```python
import os as _os
_os.environ.setdefault("JAX_PLATFORMS", "cpu")
import jax
import jax.numpy as jnp

def _softmax(x, axis=-1):
    return jax.nn.softmax(x, axis=axis)
def _gelu(x):
    return jax.nn.gelu(x, approximate=True)
def _silu(x):
    return jax.nn.silu(x)
def _sigmoid(x):
    return jax.nn.sigmoid(x)
def _layernorm(x, axis=-1, eps=1e-5):
    m = jnp.mean(x, axis=axis, keepdims=True)
    v = jnp.var(x, axis=axis, keepdims=True)
    return (x - m) / jnp.sqrt(v + eps)
def _scatter_add(tgt, idx, src, axis=0):
    return tgt.at[idx].add(src)
def _segment_sum(src, seg, n):
    return jax.ops.segment_sum(src, seg, n)
class _Rng:
    def __init__(self, key):
        self._k = key
    def _next(self):
        self._k, sub = jax.random.split(self._k)
        return sub
    def normal(self, shape):
        return jax.random.normal(self._next(), shape, dtype=jnp.bfloat16)
    def randint(self, lo, hi, shape):
        return jax.random.randint(self._next(), shape, lo, hi, dtype=jnp.int32)
    def uniform(self, shape, lo=0.0, hi=1.0):
        return jax.random.uniform(self._next(), shape, jnp.bfloat16, lo, hi)
    def permutation(self, n):
        return jax.random.permutation(self._next(), n)


kernel_name = 'standalone__mha_softmax__near_ridge'

def setup_inputs():
    _rng = _Rng(jax.random.key(int.from_bytes(__import__("os").urandom(4), "little")))
    _w = (lambda a: (lambda t: t.astype(jnp.bfloat16) if jnp.issubdtype(t.dtype, jnp.floating) else t)(jnp.asarray(a)))
    B, H, Sq, Sk, D = 8, 32, 512, 512, 128
    return {
        "q": _w((lambda *s: _rng.normal(s) * 0.4)(B, H, Sq, D)),
        "k": _w((lambda *s: _rng.normal(s) * 0.4)(B, H, Sk, D)),
        "v": _w((lambda *s: _rng.normal(s) * 0.05)(B, H, Sk, D)),
    }

def reference(q, k, v):
    scale = q.shape[-1] ** -0.5
    scores = jnp.einsum("bhqd,bhkd->bhqk", q, k) * scale
    p = _softmax(scores, axis=-1)
    return jnp.einsum("bhqk,bhkd->bhqd", p, v)
```

```python
import functools
import math

import jax
import jax.numpy as jnp
import jax.experimental.pallas as pl
import jax.experimental.pallas.tpu as pltpu


def _attn_kernel(q_ref, k_ref, v_ref, o_ref, *, scale):
    q = q_ref[0]
    k = k_ref[0]
    v = v_ref[0]
    s = jax.lax.dot_general(q, k, (((1,), (1,)), ((), ())),
                            preferred_element_type=jnp.float32)
    m = jnp.max(s, axis=-1, keepdims=True)
    p = jnp.exp((s - m) * scale)
    l = jnp.sum(p, axis=-1, keepdims=True)
    o = jnp.dot(p.astype(jnp.bfloat16), v, preferred_element_type=jnp.float32)
    o_ref[0] = (o / l).astype(o_ref.dtype)


@jax.jit
def pallas_standalone__mha_softmax__near_ridge_kernel(
    q: jax.Array,
    k: jax.Array,
    v: jax.Array,
):
    B, H, Sq, D = q.shape
    Sk = k.shape[2]
    scale = D ** -0.5
    q3 = q.reshape(B * H, Sq, D)
    k3 = k.reshape(B * H, Sk, D)
    v3 = v.reshape(B * H, Sk, D)
    out = pl.pallas_call(
        functools.partial(_attn_kernel, scale=scale),
        grid=(B * H,),
        in_specs=[
            pl.BlockSpec((1, Sq, D), lambda i: (i, 0, 0)),
            pl.BlockSpec((1, Sk, D), lambda i: (i, 0, 0)),
            pl.BlockSpec((1, Sk, D), lambda i: (i, 0, 0)),
        ],
        out_specs=pl.BlockSpec((1, Sq, D), lambda i: (i, 0, 0)),
        out_shape=jax.ShapeDtypeStruct((B * H, Sq, D), q.dtype),
        compiler_params=pltpu.CompilerParams(
            dimension_semantics=("parallel",),
        ),
    )(q3, k3, v3)
    return out.reshape(B, H, Sq, D)
```

```python
import functools

import jax
import jax.numpy as jnp
from jax import lax
import jax.experimental.pallas as pl
import jax.experimental.pallas.tpu as pltpu

_LOG2E = 1.4426950408889634
_NT = (((1,), (1,)), ((), ()))
_LANES = 128

_SEGMENTS = ((1, 2, 2), (2, 1, 3), (4, 3, 6), (8, 2, 11), (16, 14, 22))
_RING = 128
_FIRST_READS = 6
_ALT_FROM_SEG = 4
_READ_SPLIT = 2
_WRITE_FROM = 180
_WRITES_PER_HEAD = 4


def _attn_kernel(q_hbm, k_hbm, v_hbm, o_hbm, ib, ob, pbuf, sem, *, scale):
    n_heads, seq, _ = q_hbm.shape
    c = scale * _LOG2E
    rows = seq // _READ_SPLIT
    hbms = (q_hbm, k_hbm, v_hbm)
    segs = _SEGMENTS

    starts, gbase = [], []
    h = ng = 0
    for size, count, _ in segs:
        starts.append(h)
        gbase.append(ng)
        h += size * count
        ng += count
    assert h == n_heads and n_heads <= 2 * _RING
    write_sem = ng

    def group_of(j, lo, hi):
        res = None
        for s0, g0, (size, count, _) in zip(starts, gbase, segs):
            if s0 + size * count <= lo or s0 >= hi:
                continue
            if isinstance(j, int):
                res = g0 + (j - s0) // size
            else:
                g = g0 + lax.div(j - s0, size)
                res = g if res is None else jnp.where(j >= s0, g, res)
        return res

    def slot_of(j, lo, hi):
        if hi <= _RING:
            return j
        if lo >= _RING:
            return j - _RING
        return jnp.where(j >= _RING, j - _RING, j)

    def start_reads(j, lo, hi, alternate):
        if isinstance(j, int):
            lo, hi = j, j + 1
        group, slot = group_of(j, lo, hi), slot_of(j, lo, hi)
        n = 0
        for part in range(_READ_SPLIT):
            rs = pl.ds(part * rows, rows)
            for a in (1, 0, 2):
                pltpu.make_async_copy(hbms[a].at[j, rs], ib.at[slot, a, rs], sem.at[group]).start(
                    priority=n % 2 if alternate else 0)
                n += 1

    def start_write(j, priority):
        pltpu.make_async_copy(ob.at[j], o_hbm.at[j], sem.at[write_sem]).start(priority=priority)

    ib32 = ib.bitcast(jnp.uint32)
    pb32 = pbuf.bitcast(jnp.uint32)

    def load(slot, a):
        return pltpu.bitcast(ib32[slot, a], jnp.bfloat16)

    def head(q, k, v, u, j):
        s = lax.dot_general(q, k, _NT, preferred_element_type=jnp.float32)
        m = jnp.max(s, axis=-1, keepdims=True)
        p = jnp.exp2((s - m) * c)
        l = jnp.sum(p, axis=-1, keepdims=True)
        tiles = seq // _LANES
        for t in range(tiles):
            pbuf[u, t] = p[:, t * _LANES:(t + 1) * _LANES].astype(jnp.bfloat16)
        pb = jnp.concatenate([pltpu.bitcast(pb32[u, t], jnp.bfloat16) for t in range(tiles)], axis=1)
        o = jnp.dot(pb, v, preferred_element_type=jnp.float32)
        ob[j] = (o * pl.reciprocal(l, approx=True)).astype(ob.dtype)

    def written_before(j, mx, mn):
        return mx(mn(_WRITES_PER_HEAD * (j - _WRITE_FROM), j), 0)

    for j in range(_FIRST_READS):
        start_reads(j, None, None, False)

    issued = _FIRST_READS
    for si, (size, count, per_group) in enumerate(segs):
        h0 = starts[si]
        lo, hi = issued, min(n_heads, issued + count * per_group)
        for it in range(count):
            assert min(n_heads, issued + (it + 1) * per_group) - _RING <= h0 + it * size
            assert min(n_heads, issued + it * per_group) >= h0 + (it + 1) * size
            assert (h0 + it * size) % _RING + size <= _RING

        def group(it, carry, si=si, size=size, count=count, per_group=per_group, h0=h0, lo=lo, hi=hi):
            base = h0 + it * size
            rb = slot_of(base, h0, h0 + size * count)
            dst = ib.at[pl.ds(rb, size)]
            pltpu.make_async_copy(dst, dst, sem.at[gbase[si] + it]).wait()
            for g in range(size):
                j = base + g
                k = load(rb + g, 1)
                for t in range((per_group * g) // size, (per_group * (g + 1)) // size):
                    idx = lo + it * per_group + t
                    start = functools.partial(start_reads, idx, lo, hi, si >= _ALT_FROM_SEG)
                    if lo + count * per_group <= n_heads:
                        start()
                    else:
                        pl.when(idx < n_heads)(start)
                if h0 + size * count - 1 > _WRITE_FROM:
                    w0 = written_before(j - 1, jnp.maximum, jnp.minimum)
                    w1 = written_before(j, jnp.maximum, jnp.minimum)
                    for t in range(_WRITES_PER_HEAD):
                        pl.when(w0 + t < w1)(functools.partial(start_write, w0 + t, t % 2))
                head(load(rb + g, 0), k, load(rb + g, 2), g % 2, j)
            return carry

        if count == 1:
            group(0, 0)
        else:
            lax.fori_loop(0, count, group, 0)
        issued = hi
    assert issued == n_heads

    for j in range(written_before(n_heads - 1, max, min), n_heads):
        start_write(j, 0)
    pltpu.make_async_copy(ob, o_hbm, sem.at[write_sem]).wait()


@jax.jit
def pallas_standalone__mha_softmax__near_ridge_kernel(
    q: jax.Array,
    k: jax.Array,
    v: jax.Array,
):
    B, H, S, D = q.shape
    n = B * H
    n_groups = sum(count for _, count, _ in _SEGMENTS)
    out = pl.pallas_call(
        functools.partial(_attn_kernel, scale=D ** -0.5),
        in_specs=[pl.BlockSpec(memory_space=pl.ANY)] * 3,
        out_specs=pl.BlockSpec(memory_space=pl.ANY),
        out_shape=jax.ShapeDtypeStruct((n, S, D), q.dtype),
        scratch_shapes=[
            pltpu.VMEM((_RING, 3, S, D), q.dtype),
            pltpu.VMEM((n, S, D), q.dtype),
            pltpu.VMEM((2, S // _LANES, S, _LANES), q.dtype),
            pltpu.SemaphoreType.DMA((n_groups + 1,)),
        ],
        compiler_params=pltpu.CompilerParams(
            vmem_limit_bytes=110 * 1024 * 1024,
            disable_bounds_checks=True,
            disable_semaphore_checks=True,
        ),
    )(q.reshape(n, S, D), k.reshape(n, S, D), v.reshape(n, S, D))
    return out.reshape(B, H, S, D)
```

```python
import functools

import jax
import jax.numpy as jnp
from jax import lax
import jax.experimental.pallas as pl
import jax.experimental.pallas.tpu as pltpu

_LOG2E = 1.4426950408889634
_NT = (((1,), (1,)), ((), ()))
_LANES = 128

_SEGMENTS = ((1, 2, 2), (2, 2, 3), (4, 3, 5), (8, 5, 11), (22, 9, 31))
_RING = 146
_FIRST_READS = 5
_ALT_FROM_SEG = 3
_READ_SPLIT = 4
_WRITE_FROM = 180
_WRITES_PER_HEAD = 4


def _attn_kernel(q_hbm, k_hbm, v_hbm, o_hbm, ib, ob, pbuf, sem, *, scale):
    n_heads, seq, _ = q_hbm.shape
    c = scale * _LOG2E
    hbms = (q_hbm, k_hbm, v_hbm)
    segs = _SEGMENTS

    starts, gbase = [], []
    h = ng = 0
    for size, count, _ in segs:
        starts.append(h)
        gbase.append(ng)
        h += size * count
        ng += count
    assert h == n_heads and n_heads <= 2 * _RING
    write_sem = ng

    def group_of(j, lo, hi):
        res = None
        for s0, g0, (size, count, _) in zip(starts, gbase, segs):
            if s0 + size * count <= lo or s0 >= hi:
                continue
            if isinstance(j, int):
                res = g0 + (j - s0) // size
            else:
                g = g0 + lax.div(j - s0, size)
                res = g if res is None else jnp.where(j >= s0, g, res)
        return res

    def slot_of(j, lo, hi):
        if hi <= _RING:
            return j
        if lo >= _RING:
            return j - _RING
        return jnp.where(j >= _RING, j - _RING, j)

    def start_reads(j, lo, hi, alternate):
        if isinstance(j, int):
            lo, hi = j, j + 1
        group, slot = group_of(j, lo, hi), slot_of(j, lo, hi)
        split = _READ_SPLIT if alternate else 1
        rows = seq // split
        for part in range(split):
            rs = pl.ds(part * rows, rows)
            for a, priority in ((1, 1), (0, 1), (2, 0)):
                pltpu.make_async_copy(hbms[a].at[j, rs], ib.at[slot, a, rs], sem.at[group]).start(
                    priority=priority if alternate else 0)

    def start_write(j, priority):
        pltpu.make_async_copy(ob.at[j], o_hbm.at[j], sem.at[write_sem]).start(priority=priority)

    ib32 = ib.bitcast(jnp.uint32)
    pb32 = pbuf.bitcast(jnp.uint32)

    def load(slot, a):
        return pltpu.bitcast(ib32[slot, a], jnp.bfloat16)

    def head(q, k, v, u, j):
        s = lax.dot_general(q, k, _NT, preferred_element_type=jnp.float32)
        m = jnp.max(s, axis=-1, keepdims=True)
        p = jnp.exp2((s - m) * c)
        l = jnp.sum(p, axis=-1, keepdims=True)
        tiles = seq // _LANES
        for t in range(tiles):
            pbuf[u, t] = p[:, t * _LANES:(t + 1) * _LANES].astype(jnp.bfloat16)
        pb = jnp.concatenate([pltpu.bitcast(pb32[u, t], jnp.bfloat16) for t in range(tiles)], axis=1)
        o = jnp.dot(pb, v, preferred_element_type=jnp.float32)
        ob[j] = (o * pl.reciprocal(l, approx=True)).astype(ob.dtype)

    def written_before(j, mx, mn):
        return mx(mn(_WRITES_PER_HEAD * (j - _WRITE_FROM), j), 0)

    for j in range(_FIRST_READS):
        start_reads(j, None, None, False)

    issued = _FIRST_READS
    for si, (size, count, per_group) in enumerate(segs):
        h0 = starts[si]
        lo, hi = issued, min(n_heads, issued + count * per_group)
        for it in range(count):
            assert min(n_heads, issued + (it + 1) * per_group) - _RING <= h0 + it * size
            assert min(n_heads, issued + it * per_group) >= h0 + (it + 1) * size
            assert (h0 + it * size) % _RING + size <= _RING

        def group(it, carry, si=si, size=size, count=count, per_group=per_group, h0=h0, lo=lo, hi=hi):
            base = h0 + it * size
            rb = slot_of(base, h0, h0 + size * count)
            dst = ib.at[pl.ds(rb, size)]
            pltpu.make_async_copy(dst, dst, sem.at[gbase[si] + it]).wait()
            for g in range(size):
                j = base + g
                k = load(rb + g, 1)
                for t in range((per_group * g) // size, (per_group * (g + 1)) // size):
                    idx = lo + it * per_group + t
                    start = functools.partial(start_reads, idx, lo, hi, si >= _ALT_FROM_SEG)
                    if lo + count * per_group <= n_heads:
                        start()
                    else:
                        pl.when(idx < n_heads)(start)
                if h0 + size * count - 1 > _WRITE_FROM:
                    w0 = written_before(j - 1, jnp.maximum, jnp.minimum)
                    w1 = written_before(j, jnp.maximum, jnp.minimum)
                    for t in range(_WRITES_PER_HEAD):
                        pl.when(w0 + t < w1)(functools.partial(start_write, w0 + t, t % 2))
                head(load(rb + g, 0), k, load(rb + g, 2), g % 2, j)
            return carry

        if count == 1:
            group(0, 0)
        else:
            lax.fori_loop(0, count, group, 0)
        issued = hi
    assert issued == n_heads

    for j in range(written_before(n_heads - 1, max, min), n_heads):
        start_write(j, 0)
    pltpu.make_async_copy(ob, o_hbm, sem.at[write_sem]).wait()


@jax.jit
def pallas_standalone__mha_softmax__near_ridge_kernel(
    q: jax.Array,
    k: jax.Array,
    v: jax.Array,
):
    B, H, S, D = q.shape
    n = B * H
    n_groups = sum(count for _, count, _ in _SEGMENTS)
    out = pl.pallas_call(
        functools.partial(_attn_kernel, scale=D ** -0.5),
        in_specs=[pl.BlockSpec(memory_space=pl.ANY)] * 3,
        out_specs=pl.BlockSpec(memory_space=pl.ANY),
        out_shape=jax.ShapeDtypeStruct((n, S, D), q.dtype),
        scratch_shapes=[
            pltpu.VMEM((_RING, 3, S, D), q.dtype),
            pltpu.VMEM((n, S, D), q.dtype),
            pltpu.VMEM((2, S // _LANES, S, _LANES), q.dtype),
            pltpu.SemaphoreType.DMA((n_groups + 1,)),
        ],
        compiler_params=pltpu.CompilerParams(
            vmem_limit_bytes=110 * 1024 * 1024,
            disable_bounds_checks=True,
            disable_semaphore_checks=True,
        ),
    )(q.reshape(n, S, D), k.reshape(n, S, D), v.reshape(n, S, D))
    return out.reshape(B, H, S, D)
```

```python
import functools

import jax
import jax.numpy as jnp
from jax import lax
import jax.experimental.pallas as pl
import jax.experimental.pallas.tpu as pltpu

_LOG2E = 1.4426950408889634
_NT = (((1,), (1,)), ((), ()))
_LANES = 128

_SEGMENTS = ((1, 1, 2), (1, 2, 2), (2, 1, 3), (3, 1, 4), (4, 2, 5), (7, 2, 9), (11, 4, 15), (26, 7, 36))
_RING = 152
_FIRST_READS = 4
_READ_SPLIT = 4
_REGIONS = 4
_WRITE_ROWS = 128
_WRITE_FROM = 186
_WRITES_PER_HEAD = 4
_WRITE_EVERY = 2
_CARRY_ROWS = 128


def _shift(x, pow2):
    if isinstance(x, int):
        return x // pow2
    return lax.shift_right_arithmetic(x, pow2.bit_length() - 1)


def _attn_kernel(q_hbm, k_hbm, v_hbm, o_hbm, ib, ob, pbuf, pcar, rcar, vcar, sem, *, scale):
    regions, per_region, seq, _ = q_hbm.shape
    n_heads = regions * per_region
    tiles = seq // _LANES
    keep = seq - _CARRY_ROWS
    c = scale * _LOG2E
    hbms = (q_hbm, k_hbm, v_hbm)
    segs = _SEGMENTS

    starts, gbase = [], []
    h = n_groups = 0
    for size, count, _ in segs:
        starts.append(h)
        gbase.append(n_groups)
        h += size * count
        n_groups += count
    assert h == n_heads <= 2 * _RING and segs[0][1] == 1
    write_sem = sem.at[n_groups]

    def where_is(j):
        return j & (regions - 1), _shift(j, regions)

    def group_of(j, lo, hi):
        res = None
        for s0, g0, (size, count, _) in zip(starts, gbase, segs):
            if s0 + size * count <= lo or s0 >= hi:
                continue
            magic = -(-(1 << 16) // size)
            assert all((x * magic) >> 16 == x // size for x in range(n_heads))
            g = g0 + _shift((j - s0) * magic, 1 << 16)
            res = g if res is None else jnp.where(j >= s0, g, res)
        return res

    def slot_of(j, lo, hi):
        if hi <= _RING:
            return j
        if lo >= _RING:
            return j - _RING
        return jnp.where(j >= _RING, j - _RING, j)

    def start_reads(j, lo, hi, part, split):
        if isinstance(j, int):
            lo, hi = j, j + 1
        group, slot = group_of(j, lo, hi), slot_of(j, lo, hi)
        r, i = where_is(j)
        rows = pl.ds(part * (seq // split), seq // split)
        for a, priority in ((1, 1), (0, 1), (2, 0)):
            pltpu.make_async_copy(hbms[a].at[r, i, rows], ib.at[slot, a, rows], sem.at[group]).start(
                priority=priority if split > 1 else 0)

    chunks = seq // _WRITE_ROWS
    n_bulk = (per_region - 1) * chunks

    def start_bulk_write(u):
        i = _shift(u, chunks)
        row0 = (u & (chunks - 1)) * _WRITE_ROWS
        if not isinstance(row0, int):
            row0 = pl.multiple_of(row0, _WRITE_ROWS)
        rows = pl.ds(row0, _WRITE_ROWS)
        pltpu.make_async_copy(ob.at[i, :, rows], o_hbm.at[:, i, rows], write_sem).start()

    def start_head_write(j, row0=0, n=seq):
        r, i = where_is(j)
        rows = pl.ds(row0, n)
        pltpu.make_async_copy(ob.at[i, r, rows], o_hbm.at[r, i, rows], write_sem).start()

    def bulk_before(j):
        mx, mn = (max, min) if isinstance(j, int) else (jnp.maximum, jnp.minimum)
        return mx(mn(mn(_WRITES_PER_HEAD * (j - _WRITE_FROM), _shift(j, regions) * chunks), n_bulk), 0)

    ib32 = ib.bitcast(jnp.uint32)
    pb32 = pbuf.bitcast(jnp.uint32)
    pc32 = pcar.bitcast(jnp.uint32)

    def as_bf16(x):
        return pltpu.bitcast(x, jnp.bfloat16)

    def head(q, k, v32, u, j, last):
        n = keep if last else seq
        r, i = where_is(j)
        s = lax.dot_general(q, k, _NT, preferred_element_type=jnp.float32)
        m = jnp.max(s, axis=-1, keepdims=True)
        p = jnp.exp2((s - m) * c)
        inv = pl.reciprocal(jnp.sum(p, axis=-1, keepdims=True), approx=True)
        for t in range(tiles):
            cols = slice(t * _LANES, (t + 1) * _LANES)
            pbuf[u, t, pl.ds(0, n)] = p[:n, cols].astype(pbuf.dtype)
            if last:
                pcar[t] = p[n:, cols].astype(pcar.dtype)
        if last:
            rcar[...] = jnp.broadcast_to(inv[n:], rcar.shape)
            vcar[...] = v32
        pb = jnp.concatenate([as_bf16(pb32[u, t, pl.ds(0, n // 2)]) for t in range(tiles)], axis=1)
        o = jnp.dot(pb, as_bf16(v32), preferred_element_type=jnp.float32)
        ob[i, r, pl.ds(0, n)] = (o * inv[:n]).astype(ob.dtype)

    def finish_head(j):
        r, i = where_is(j)
        pb = jnp.concatenate([as_bf16(pc32[t]) for t in range(tiles)], axis=1)
        o = jnp.dot(pb, as_bf16(vcar[...]), preferred_element_type=jnp.float32)
        ob[i, r, pl.ds(keep, _CARRY_ROWS)] = (o * rcar[...]).astype(ob.dtype)

    def run_segment(si, lo):
        size, count, per_group = segs[si]
        h0 = starts[si]
        hi = min(n_heads, lo + count * per_group)
        final = si == len(segs) - 1
        split = _READ_SPLIT if final else 1
        assert final or h0 + size * count <= _WRITE_FROM
        for it in range(count):
            assert min(n_heads, lo + (it + 1) * per_group) - _RING <= h0 + it * size
            assert min(n_heads, lo + it * per_group) >= h0 + (it + 1) * size
            assert (h0 + it * size) % _RING + size <= _RING

        def group(it, slot0):
            base = h0 + it * size
            dst = ib.at[pl.ds(slot0, size)]
            pltpu.make_async_copy(dst, dst, sem.at[gbase[si] + it]).wait()
            if h0 > 0:
                finish_head(base - 1)
            for g in range(size):
                j, slot = base + g, slot0 + g
                reads = []
                for t in range((per_group * g) // size, (per_group * (g + 1)) // size):
                    idx = lo + it * per_group + t
                    for part in range(split):
                        start = functools.partial(start_reads, idx, lo, hi, part, split)
                        if lo + count * per_group > n_heads:
                            start = functools.partial(pl.when(idx < n_heads), start)
                        reads.append(start)
                k = as_bf16(ib32[slot, 1])
                for start in reads[:len(reads) // 2]:
                    start()
                if final and (size - 1 - g) % _WRITE_EVERY == 0:
                    back = min(_WRITE_EVERY, g + 1)
                    w0, w1 = bulk_before(j - back), bulk_before(j)
                    for t in range(max(_WRITES_PER_HEAD * back, chunks)):
                        pl.when(w0 + t < w1)(functools.partial(start_bulk_write, w0 + t))
                    for done in range(n_heads - size + g - back, n_heads - size + g):
                        if done >= n_heads - regions:
                            pl.when(it == count - 1)(functools.partial(start_head_write, done))
                v32 = ib32[slot, 2]
                q_top = as_bf16(ib32[slot, 0, pl.ds(0, seq // 4)])
                for start in reads[len(reads) // 2:]:
                    start()
                q_bottom = as_bf16(ib32[slot, 0, pl.ds(seq // 4, seq // 4)])
                head(jnp.concatenate([q_top, q_bottom], axis=0), k, v32, g % 2, j, g == size - 1)
            return slot_of(base + size, h0 + size, h0 + size * (count + 1))

        if count == 1:
            group(0, h0 % _RING)
        else:
            lax.fori_loop(0, count, group, h0 % _RING)
        return hi

    @pl.when(pl.program_id(0) == 0)
    def _():
        for j in range(_FIRST_READS):
            start_reads(j, None, None, 0, 1)

    @pl.when(pl.program_id(0) == 1)
    def _():
        issued = _FIRST_READS
        for si in range(len(segs)):
            issued = run_segment(si, issued)
        assert issued == n_heads and bulk_before(n_heads - 1) == n_bulk
        start_head_write(n_heads - 1, 0, keep)
        finish_head(n_heads - 1)
        start_head_write(n_heads - 1, keep, _CARRY_ROWS)
        pltpu.make_async_copy(ob, ob, write_sem).wait()


@jax.jit
def pallas_standalone__mha_softmax__near_ridge_kernel(
    q: jax.Array,
    k: jax.Array,
    v: jax.Array,
):
    B, H, S, D = q.shape
    per_region = B * H // _REGIONS
    shape = (_REGIONS, per_region, S, D)
    n_groups = sum(count for _, count, _ in _SEGMENTS)
    out = pl.pallas_call(
        functools.partial(_attn_kernel, scale=D ** -0.5),
        grid=(2,),
        in_specs=[pl.BlockSpec(memory_space=pl.ANY)] * 3,
        out_specs=pl.BlockSpec(memory_space=pl.ANY),
        out_shape=jax.ShapeDtypeStruct(shape, q.dtype),
        scratch_shapes=[
            pltpu.VMEM((_RING, 3, S, D), q.dtype),
            pltpu.VMEM((per_region, _REGIONS, S, D), q.dtype),
            pltpu.VMEM((2, S // _LANES, S, _LANES), q.dtype),
            pltpu.VMEM((S // _LANES, _CARRY_ROWS, _LANES), q.dtype),
            pltpu.VMEM((_CARRY_ROWS, D), jnp.float32),
            pltpu.VMEM((S // 2, D), jnp.uint32),
            pltpu.SemaphoreType.DMA((n_groups + 1,)),
        ],
        compiler_params=pltpu.CompilerParams(
            dimension_semantics=("arbitrary",),
            vmem_limit_bytes=110 * 1024 * 1024,
            disable_bounds_checks=True,
            disable_semaphore_checks=True,
        ),
    )(q.reshape(shape), k.reshape(shape), v.reshape(shape))
    return out.reshape(B, H, S, D)
```

```python
import functools

import jax
import jax.numpy as jnp
from jax import lax
import jax.experimental.pallas as pl
import jax.experimental.pallas.tpu as pltpu

_LOG2E = 1.4426950408889634
_NT = (((1,), (1,)), ((), ()))
_LANES = 128

_SEGMENTS = ((1, 1, 2), (1, 2, 2), (2, 1, 3), (3, 1, 4), (4, 2, 6), (6, 2, 9), (12, 4, 17), (30, 6, 41))
_RING = 136
_FIRST_READS = 3
_SPLIT_FROM = 4
_READ_SPLIT = 4
_V_LAG = 3
_REGIONS = 4
_WRITE_ROWS = 128
_WRITE_FROM = 186
_WRITES_PER_HEAD = 4
_WRITE_EVERY = 2
_CARRY_ROWS = 128


def _shift(x, pow2):
    if isinstance(x, int):
        return x // pow2
    return lax.shift_right_arithmetic(x, pow2.bit_length() - 1)


def _attn_kernel(q_hbm, k_hbm, v_hbm, o_hbm, ib, ob, pbuf, pcar, rcar, vcar, sem, *, scale):
    regions, per_region, seq, _ = q_hbm.shape
    n_heads = regions * per_region
    tiles = seq // _LANES
    keep = seq - _CARRY_ROWS
    c = scale * _LOG2E
    hbms = (q_hbm, k_hbm, v_hbm)
    segs = _SEGMENTS

    starts, gbase = [], []
    h = n_groups = 0
    for size, count, _ in segs:
        starts.append(h)
        gbase.append(n_groups)
        h += size * count
        n_groups += count
    assert h == n_heads <= 2 * _RING and segs[0][1] == 1
    write_sem = sem.at[n_groups]
    first_split = _FIRST_READS + sum(count * per_group for _, count, per_group in segs[:_SPLIT_FROM])

    def where_is(j):
        return j & (regions - 1), _shift(j, regions)

    def group_of(j, lo, hi):
        res = None
        for s0, g0, (size, count, _) in zip(starts, gbase, segs):
            if s0 + size * count <= lo or s0 >= hi:
                continue
            magic = -(-(1 << 16) // size)
            assert all((x * magic) >> 16 == x // size for x in range(n_heads))
            g = g0 + _shift((j - s0) * magic, 1 << 16)
            res = g if res is None else jnp.where(j >= s0, g, res)
        return res

    def slot_of(j, lo, hi):
        if hi <= _RING:
            return j
        if lo >= _RING:
            return j - _RING
        return jnp.where(j >= _RING, j - _RING, j)

    def start_reads(arrays, j, lo, hi, part=0, split=1, priority=0):
        first = first_split if split > 1 else 0
        if isinstance(j, int):
            lo, hi = j, j + 1

        def start():
            group, slot = group_of(j, max(lo, first), min(hi, n_heads)), slot_of(j, lo, hi)
            r, i = where_is(j)
            rows = pl.ds(part * (seq // split), seq // split)
            for a in arrays:
                pltpu.make_async_copy(hbms[a].at[r, i, rows], ib.at[slot, a, rows], sem.at[group]).start(
                    priority=priority)

        if first <= lo and hi <= n_heads:
            start()
        elif not isinstance(j, int):
            pl.when(jnp.logical_and(j >= first, j < n_heads))(start)

    def start_part(j, lo, hi, part):
        start_reads((1, 0), j, lo, hi, part, _READ_SPLIT, 1)
        start_reads((2,), j - _V_LAG, lo - _V_LAG, hi - _V_LAG, part, _READ_SPLIT, 0)

    chunks = seq // _WRITE_ROWS
    n_bulk = (per_region - 1) * chunks

    def start_bulk_write(u):
        i = _shift(u, chunks)
        row0 = (u & (chunks - 1)) * _WRITE_ROWS
        if not isinstance(row0, int):
            row0 = pl.multiple_of(row0, _WRITE_ROWS)
        rows = pl.ds(row0, _WRITE_ROWS)
        pltpu.make_async_copy(ob.at[i, :, rows], o_hbm.at[:, i, rows], write_sem).start()

    def start_head_write(j, row0=0, n=seq):
        r, i = where_is(j)
        rows = pl.ds(row0, n)
        pltpu.make_async_copy(ob.at[i, r, rows], o_hbm.at[r, i, rows], write_sem).start()

    def bulk_before(j):
        mx, mn = (max, min) if isinstance(j, int) else (jnp.maximum, jnp.minimum)
        return mx(mn(mn(_WRITES_PER_HEAD * (j - _WRITE_FROM), _shift(j, regions) * chunks), n_bulk), 0)

    def load_words(view):
        return view.bitcast(jnp.uint32)[...]

    def as_bf16(x):
        return pltpu.bitcast(x, jnp.bfloat16)

    def load(view):
        return as_bf16(load_words(view))

    def head(q, k, v32, u, j, last):
        n = keep if last else seq
        r, i = where_is(j)
        s = lax.dot_general(q, k, _NT, preferred_element_type=jnp.float32)
        m = jnp.max(s, axis=-1, keepdims=True)
        p = jnp.exp2((s - m) * c)
        inv = pl.reciprocal(jnp.sum(p, axis=-1, keepdims=True), approx=True)
        for t in range(tiles):
            cols = slice(t * _LANES, (t + 1) * _LANES)
            pbuf[u, t, pl.ds(0, n)] = p[:n, cols].astype(pbuf.dtype)
            if last:
                pcar[t] = p[n:, cols].astype(pcar.dtype)
        if last:
            rcar[...] = jnp.broadcast_to(inv[n:], rcar.shape)
            vcar[...] = v32
        pb = jnp.concatenate([load(pbuf.at[u, t, pl.ds(0, n)]) for t in range(tiles)], axis=1)
        o = jnp.dot(pb, as_bf16(v32), preferred_element_type=jnp.float32)
        ob[i, r, pl.ds(0, n)] = (o * inv[:n]).astype(ob.dtype)

    def finish_head(j):
        r, i = where_is(j)
        pb = jnp.concatenate([load(pcar.at[t]) for t in range(tiles)], axis=1)
        o = jnp.dot(pb, as_bf16(vcar[...]), preferred_element_type=jnp.float32)
        ob[i, r, pl.ds(keep, _CARRY_ROWS)] = (o * rcar[...]).astype(ob.dtype)

    def run_segment(si, lo):
        size, count, per_group = segs[si]
        h0 = starts[si]
        hi = lo + count * per_group
        final = si == len(segs) - 1
        assert final or h0 + size * count <= _WRITE_FROM
        for it in range(count):
            issued = lo + it * per_group
            assert min(n_heads, issued + per_group) - _RING <= h0 + it * size
            assert min(issued, max(issued - _V_LAG, first_split)) >= h0 + (it + 1) * size
            assert (h0 + it * size) % _RING + size <= _RING

        def group(it, slot0):
            base = h0 + it * size
            dst = ib.at[pl.ds(slot0, size)]
            pltpu.make_async_copy(dst, dst, sem.at[gbase[si] + it]).wait()
            if h0 > 0:
                finish_head(base - 1)
            for g in range(size):
                j, slot = base + g, slot0 + g
                reads = []
                for t in range((per_group * g) // size, (per_group * (g + 1)) // size):
                    idx = lo + it * per_group + t
                    if si < _SPLIT_FROM:
                        reads.append(functools.partial(start_reads, (1, 0, 2), idx, lo, hi))
                    else:
                        reads += [functools.partial(start_part, idx, lo, hi, part) for part in range(_READ_SPLIT)]
                k = load(ib.at[slot, 1])
                for start in reads[:len(reads) // 2]:
                    start()
                if final and (size - 1 - g) % _WRITE_EVERY == 0:
                    back = min(_WRITE_EVERY, g + 1)
                    w0, w1 = bulk_before(j - back), bulk_before(j)
                    for t in range(max(_WRITES_PER_HEAD * back, chunks)):
                        pl.when(w0 + t < w1)(functools.partial(start_bulk_write, w0 + t))
                    for done in range(n_heads - size + g - back, n_heads - size + g):
                        if done >= n_heads - regions:
                            pl.when(it == count - 1)(functools.partial(start_head_write, done))
                v32 = load_words(ib.at[slot, 2])
                q_top = load(ib.at[slot, 0, pl.ds(0, seq // 2)])
                for start in reads[len(reads) // 2:]:
                    start()
                q_bottom = load(ib.at[slot, 0, pl.ds(seq // 2, seq // 2)])
                head(jnp.concatenate([q_top, q_bottom], axis=0), k, v32, g % 2, j, g == size - 1)
            return slot_of(base + size, h0 + size, h0 + size * (count + 1))

        if count == 1:
            group(0, h0 % _RING)
        else:
            lax.fori_loop(0, count, group, h0 % _RING)
        return hi

    @pl.when(pl.program_id(0) == 0)
    def _():
        for j in range(_FIRST_READS):
            start_reads((1, 0, 2), j, None, None)

    @pl.when(pl.program_id(0) == 1)
    def _():
        issued = _FIRST_READS
        for si in range(len(segs)):
            issued = run_segment(si, issued)
        assert issued - _V_LAG >= n_heads and bulk_before(n_heads - 1) == n_bulk
        start_head_write(n_heads - 1, 0, keep)
        finish_head(n_heads - 1)
        start_head_write(n_heads - 1, keep, _CARRY_ROWS)
        pltpu.make_async_copy(o_hbm, o_hbm, write_sem).wait()


@jax.jit
def pallas_standalone__mha_softmax__near_ridge_kernel(
    q: jax.Array,
    k: jax.Array,
    v: jax.Array,
):
    B, H, S, D = q.shape
    per_region = B * H // _REGIONS
    shape = (_REGIONS, per_region, S, D)
    n_groups = sum(count for _, count, _ in _SEGMENTS)
    out = pl.pallas_call(
        functools.partial(_attn_kernel, scale=D ** -0.5),
        grid=(2,),
        in_specs=[pl.BlockSpec(memory_space=pl.ANY)] * 3,
        out_specs=pl.BlockSpec(memory_space=pl.ANY),
        out_shape=jax.ShapeDtypeStruct(shape, q.dtype),
        scratch_shapes=[
            pltpu.VMEM((_RING, 3, S, D), q.dtype),
            pltpu.VMEM((per_region, _REGIONS, S, D), q.dtype),
            pltpu.VMEM((2, S // _LANES, S, _LANES), q.dtype),
            pltpu.VMEM((S // _LANES, _CARRY_ROWS, _LANES), q.dtype),
            pltpu.VMEM((_CARRY_ROWS, D), jnp.float32),
            pltpu.VMEM((S // 2, D), jnp.uint32),
            pltpu.SemaphoreType.DMA((n_groups + 1,)),
        ],
        compiler_params=pltpu.CompilerParams(
            dimension_semantics=("arbitrary",),
            vmem_limit_bytes=110 * 1024 * 1024,
            disable_bounds_checks=True,
            disable_semaphore_checks=True,
        ),
    )(q.reshape(shape), k.reshape(shape), v.reshape(shape))
    return out.reshape(B, H, S, D)
```

```python
import functools

import jax
import jax.numpy as jnp
from jax import lax
import jax.experimental.pallas as pl
import jax.experimental.pallas.tpu as pltpu

_LOG2E = 1.4426950408889634
_NT = (((1,), (1,)), ((), ()))
_LANES = 128

_SEGMENTS = ((1, 1, 2), (1, 2, 2), (2, 1, 3), (3, 1, 4), (4, 2, 6), (6, 2, 9), (12, 4, 17), (30, 6, 41))
_RING = 136
_FIRST_READS = 3
_SPLIT_FROM = 4
_READ_SPLIT = 4
_V_LAG = 3
_REGIONS = 4
_WRITE_ROWS = 128
_WRITE_FROM = 184
_WRITES_PER_HEAD = 4
_WRITE_EVERY = 2
_CARRY_ROWS = 128
_LAST_PIECES = 4


def _shift(x, pow2):
    if isinstance(x, int):
        return x // pow2
    return lax.shift_right_arithmetic(x, pow2.bit_length() - 1)


def _attn_kernel(q_hbm, k_hbm, v_hbm, o_hbm, ib, ob, pbuf, pcar, rcar, vcar, sem, *, scale):
    regions, per_region, seq, _ = q_hbm.shape
    n_heads = regions * per_region
    tiles = seq // _LANES
    keep = seq - _CARRY_ROWS
    c = scale * _LOG2E
    hbms = (q_hbm, k_hbm, v_hbm)
    segs = _SEGMENTS

    starts, gbase = [], []
    h = n_groups = 0
    for size, count, _ in segs:
        starts.append(h)
        gbase.append(n_groups)
        h += size * count
        n_groups += count
    assert h == n_heads <= 2 * _RING and segs[0][1] == 1
    write_sem = sem.at[n_groups]
    first_split = _FIRST_READS + sum(count * per_group for _, count, per_group in segs[:_SPLIT_FROM])

    def where_is(j):
        return j & (regions - 1), _shift(j, regions)

    def group_of(j, lo, hi):
        res = None
        for s0, g0, (size, count, _) in zip(starts, gbase, segs):
            if s0 + size * count <= lo or s0 >= hi:
                continue
            magic = -(-(1 << 16) // size)
            assert all((x * magic) >> 16 == x // size for x in range(n_heads))
            g = g0 + _shift((j - s0) * magic, 1 << 16)
            res = g if res is None else jnp.where(j >= s0, g, res)
        return res

    def slot_of(j, lo, hi):
        if hi <= _RING:
            return j
        if lo >= _RING:
            return j - _RING
        return jnp.where(j >= _RING, j - _RING, j)

    def start_reads(arrays, j, lo, hi, part=0, split=1, priority=0):
        first = first_split if split > 1 else 0
        if isinstance(j, int):
            lo, hi = j, j + 1

        def start():
            group, slot = group_of(j, max(lo, first), min(hi, n_heads)), slot_of(j, lo, hi)
            r, i = where_is(j)
            rows = pl.ds(part * (seq // split), seq // split)
            for a in arrays:
                pltpu.make_async_copy(hbms[a].at[r, i, rows], ib.at[slot, a, rows], sem.at[group]).start(
                    priority=priority)

        if first <= lo and hi <= n_heads:
            start()
        elif not isinstance(j, int):
            pl.when(jnp.logical_and(j >= first, j < n_heads))(start)

    def start_part(j, lo, hi, part):
        start_reads((1, 0), j, lo, hi, part, _READ_SPLIT, 1)
        start_reads((2,), j - _V_LAG, lo - _V_LAG, hi - _V_LAG, part, _READ_SPLIT, 0)

    chunks = seq // _WRITE_ROWS
    n_bulk = (per_region - 1) * chunks

    def start_bulk_write(u):
        i = _shift(u, chunks)
        row0 = (u & (chunks - 1)) * _WRITE_ROWS
        if not isinstance(row0, int):
            row0 = pl.multiple_of(row0, _WRITE_ROWS)
        rows = pl.ds(row0, _WRITE_ROWS)
        pltpu.make_async_copy(ob.at[i, :, rows], o_hbm.at[:, i, rows], write_sem).start()

    def start_head_write(j, row0=0, n=seq):
        r, i = where_is(j)
        rows = pl.ds(row0, n)
        pltpu.make_async_copy(ob.at[i, r, rows], o_hbm.at[r, i, rows], write_sem).start()

    def bulk_before(j):
        mx, mn = (max, min) if isinstance(j, int) else (jnp.maximum, jnp.minimum)
        return mx(mn(mn(_WRITES_PER_HEAD * (j - _WRITE_FROM), _shift(j, regions) * chunks), n_bulk), 0)

    def load_words(view):
        return view.bitcast(jnp.uint32)[...]

    def as_bf16(x):
        return pltpu.bitcast(x, jnp.bfloat16)

    def load(view):
        return as_bf16(load_words(view))

    def head(q, k, v32, u, j, last):
        n = keep if last else seq
        r, i = where_is(j)
        s = lax.dot_general(q, k, _NT, preferred_element_type=jnp.float32)
        m = jnp.max(s, axis=-1, keepdims=True)
        p = jnp.exp2((s - m) * c)
        inv = pl.reciprocal(jnp.sum(p, axis=-1, keepdims=True), approx=True)
        for t in range(tiles):
            cols = slice(t * _LANES, (t + 1) * _LANES)
            pbuf[u, t, pl.ds(0, n)] = p[:n, cols].astype(pbuf.dtype)
            if last:
                pcar[t] = p[n:, cols].astype(pcar.dtype)
        if last:
            rcar[...] = jnp.broadcast_to(inv[n:], rcar.shape)
            vcar[...] = v32
        pb = jnp.concatenate([load(pbuf.at[u, t, pl.ds(0, n)]) for t in range(tiles)], axis=1)
        o = jnp.dot(pb, as_bf16(v32), preferred_element_type=jnp.float32)
        ob[i, r, pl.ds(0, n)] = (o * inv[:n]).astype(ob.dtype)

    def finish_head(j, pieces=1, after_piece=None):
        r, i = where_is(j)
        pb = jnp.concatenate([load(pcar.at[t]) for t in range(tiles)], axis=1)
        o = jnp.dot(pb, as_bf16(vcar[...]), preferred_element_type=jnp.float32)
        o = (o * rcar[...]).astype(ob.dtype)
        n = _CARRY_ROWS // pieces
        for row0 in range(0, _CARRY_ROWS, n):
            ob[i, r, pl.ds(keep + row0, n)] = o[row0:row0 + n]
            if after_piece is not None:
                after_piece(j, keep + row0, n)

    def run_segment(si, lo):
        size, count, per_group = segs[si]
        h0 = starts[si]
        hi = lo + count * per_group
        final = si == len(segs) - 1
        assert final or h0 + size * count <= _WRITE_FROM
        for it in range(count):
            issued = lo + it * per_group
            assert min(n_heads, issued + per_group) - _RING <= h0 + it * size
            assert min(issued, max(issued - _V_LAG, first_split)) >= h0 + (it + 1) * size
            assert (h0 + it * size) % _RING + size <= _RING

        def group(it, slot0):
            base = h0 + it * size
            dst = ib.at[pl.ds(slot0, size)]
            pltpu.make_async_copy(dst, dst, sem.at[gbase[si] + it]).wait()
            if h0 > 0:
                finish_head(base - 1)
            for g in range(size):
                j, slot = base + g, slot0 + g
                reads = []
                for t in range((per_group * g) // size, (per_group * (g + 1)) // size):
                    idx = lo + it * per_group + t
                    if si < _SPLIT_FROM:
                        reads.append(functools.partial(start_reads, (1, 0, 2), idx, lo, hi))
                    else:
                        reads += [functools.partial(start_part, idx, lo, hi, part) for part in range(_READ_SPLIT)]
                k = load(ib.at[slot, 1])
                for start in reads[:len(reads) // 2]:
                    start()
                if final and (size - 1 - g) % _WRITE_EVERY == 0:
                    back = min(_WRITE_EVERY, g + 1)
                    w0, w1 = bulk_before(j - back), bulk_before(j)
                    for t in range(max(_WRITES_PER_HEAD * back, chunks)):
                        pl.when(w0 + t < w1)(functools.partial(start_bulk_write, w0 + t))
                    for done in range(n_heads - size + g - back, n_heads - size + g):
                        if done >= n_heads - regions:
                            pl.when(it == count - 1)(functools.partial(start_head_write, done))
                v32 = load_words(ib.at[slot, 2])
                q_top = load(ib.at[slot, 0, pl.ds(0, seq // 2)])
                for start in reads[len(reads) // 2:]:
                    start()
                q_bottom = load(ib.at[slot, 0, pl.ds(seq // 2, seq // 2)])
                head(jnp.concatenate([q_top, q_bottom], axis=0), k, v32, g % 2, j, g == size - 1)
            return slot_of(base + size, h0 + size, h0 + size * (count + 1))

        if count == 1:
            group(0, h0 % _RING)
        else:
            lax.fori_loop(0, count, group, h0 % _RING)
        return hi

    @pl.when(pl.program_id(0) == 0)
    def _():
        for j in range(_FIRST_READS):
            start_reads((1, 0, 2), j, None, None)

    @pl.when(pl.program_id(0) == 1)
    def _():
        issued = _FIRST_READS
        for si in range(len(segs)):
            issued = run_segment(si, issued)
        assert issued - _V_LAG >= n_heads and bulk_before(n_heads - 1) == n_bulk
        start_head_write(n_heads - 1, 0, keep)
        finish_head(n_heads - 1, _LAST_PIECES, start_head_write)
        pltpu.make_async_copy(o_hbm, o_hbm, write_sem).wait()


@jax.jit
def pallas_standalone__mha_softmax__near_ridge_kernel(
    q: jax.Array,
    k: jax.Array,
    v: jax.Array,
):
    B, H, S, D = q.shape
    per_region = B * H // _REGIONS
    shape = (_REGIONS, per_region, S, D)
    n_groups = sum(count for _, count, _ in _SEGMENTS)
    out = pl.pallas_call(
        functools.partial(_attn_kernel, scale=D ** -0.5),
        grid=(2,),
        in_specs=[pl.BlockSpec(memory_space=pl.ANY)] * 3,
        out_specs=pl.BlockSpec(memory_space=pl.ANY),
        out_shape=jax.ShapeDtypeStruct(shape, q.dtype),
        scratch_shapes=[
            pltpu.VMEM((_RING, 3, S, D), q.dtype),
            pltpu.VMEM((per_region, _REGIONS, S, D), q.dtype),
            pltpu.VMEM((2, S // _LANES, S, _LANES), q.dtype),
            pltpu.VMEM((S // _LANES, _CARRY_ROWS, _LANES), q.dtype),
            pltpu.VMEM((_CARRY_ROWS, D), jnp.float32),
            pltpu.VMEM((S // 2, D), jnp.uint32),
            pltpu.SemaphoreType.DMA((n_groups + 1,)),
        ],
        compiler_params=pltpu.CompilerParams(
            dimension_semantics=("arbitrary",),
            vmem_limit_bytes=110 * 1024 * 1024,
            disable_bounds_checks=True,
            disable_semaphore_checks=True,
        ),
    )(q.reshape(shape), k.reshape(shape), v.reshape(shape))
    return out.reshape(B, H, S, D)
```

```python
import functools

import jax
import jax.numpy as jnp
from jax import lax
import jax.experimental.pallas as pl
import jax.experimental.pallas.tpu as pltpu

_LOG2E = 1.4426950408889634
_NT = (((1,), (1,)), ((), ()))
_LANES = 128

_SEGMENTS = ((1, 1, 2), (1, 2, 2), (2, 1, 3), (3, 1, 4), (4, 2, 6), (6, 2, 9), (12, 4, 17), (30, 6, 41))
_RING = 136
_FIRST_READS = 3
_SPLIT_FROM = 4
_READ_SPLIT = 4
_V_LAG = 3
_REGIONS = 4
_WRITE_ROWS = 128
_WRITE_FROM = 184
_WRITES_PER_HEAD = 4
_WRITE_EVERY = 2
_CARRY_ROWS = 128
_RAW_ROWS = 16
_LAST_PIECES = 4


def _shift(x, pow2):
    if isinstance(x, int):
        return x // pow2
    return lax.shift_right_arithmetic(x, pow2.bit_length() - 1)


def _attn_kernel(q_hbm, k_hbm, v_hbm, o_hbm, ib, ob, pbuf, pcar, rcar, vcar, ocar, sem, *, scale):
    regions, per_region, seq, _ = q_hbm.shape
    n_heads = regions * per_region
    tiles = seq // _LANES
    keep = seq - _CARRY_ROWS
    done_rows = keep - _RAW_ROWS
    c = scale * _LOG2E
    hbms = (q_hbm, k_hbm, v_hbm)
    segs = _SEGMENTS

    starts, gbase = [], []
    h = n_groups = 0
    for size, count, _ in segs:
        starts.append(h)
        gbase.append(n_groups)
        h += size * count
        n_groups += count
    assert h == n_heads <= 2 * _RING and segs[0][1] == 1
    write_sem = sem.at[n_groups]
    first_split = _FIRST_READS + sum(count * per_group for _, count, per_group in segs[:_SPLIT_FROM])

    def where_is(j):
        return j & (regions - 1), _shift(j, regions)

    def group_of(j, lo, hi):
        res = None
        for s0, g0, (size, count, _) in zip(starts, gbase, segs):
            if s0 + size * count <= lo or s0 >= hi:
                continue
            magic = -(-(1 << 16) // size)
            assert all((x * magic) >> 16 == x // size for x in range(n_heads))
            g = g0 + _shift((j - s0) * magic, 1 << 16)
            res = g if res is None else jnp.where(j >= s0, g, res)
        return res

    def slot_of(j, lo, hi):
        if hi <= _RING:
            return j
        if lo >= _RING:
            return j - _RING
        return jnp.where(j >= _RING, j - _RING, j)

    def start_reads(arrays, j, lo, hi, part=0, split=1, priority=0):
        first = first_split if split > 1 else 0
        if isinstance(j, int):
            lo, hi = j, j + 1

        def start():
            group, slot = group_of(j, max(lo, first), min(hi, n_heads)), slot_of(j, lo, hi)
            r, i = where_is(j)
            rows = pl.ds(part * (seq // split), seq // split)
            for a in arrays:
                pltpu.make_async_copy(hbms[a].at[r, i, rows], ib.at[slot, a, rows], sem.at[group]).start(
                    priority=priority)

        if first <= lo and hi <= n_heads:
            start()
        elif not isinstance(j, int):
            pl.when(jnp.logical_and(j >= first, j < n_heads))(start)

    def start_part(j, lo, hi, part):
        start_reads((1, 0), j, lo, hi, part, _READ_SPLIT, 1)
        start_reads((2,), j - _V_LAG, lo - _V_LAG, hi - _V_LAG, part, _READ_SPLIT, 0)

    chunks = seq // _WRITE_ROWS
    n_bulk = (per_region - 1) * chunks

    def start_bulk_write(u):
        i = _shift(u, chunks)
        row0 = (u & (chunks - 1)) * _WRITE_ROWS
        if not isinstance(row0, int):
            row0 = pl.multiple_of(row0, _WRITE_ROWS)
        rows = pl.ds(row0, _WRITE_ROWS)
        pltpu.make_async_copy(ob.at[i, :, rows], o_hbm.at[:, i, rows], write_sem).start()

    def start_head_write(j, row0=0, n=seq):
        r, i = where_is(j)
        rows = pl.ds(row0, n)
        pltpu.make_async_copy(ob.at[i, r, rows], o_hbm.at[r, i, rows], write_sem).start()

    def bulk_before(j):
        mx, mn = (max, min) if isinstance(j, int) else (jnp.maximum, jnp.minimum)
        return mx(mn(mn(_WRITES_PER_HEAD * (j - _WRITE_FROM), _shift(j, regions) * chunks), n_bulk), 0)

    def load_words(view):
        return view.bitcast(jnp.uint32)[...]

    def as_bf16(x):
        return pltpu.bitcast(x, jnp.bfloat16)

    def load(view):
        return as_bf16(load_words(view))

    def head(q, k, v32, u, j, last):
        n = keep if last else seq
        r, i = where_is(j)
        s = lax.dot_general(q, k, _NT, preferred_element_type=jnp.float32)
        m = jnp.max(s, axis=-1, keepdims=True)
        p = jnp.exp2((s - m) * c)
        inv = pl.reciprocal(jnp.sum(p, axis=-1, keepdims=True), approx=True)
        for t in range(tiles):
            cols = slice(t * _LANES, (t + 1) * _LANES)
            pbuf[u, t, pl.ds(0, n)] = p[:n, cols].astype(pbuf.dtype)
            if last:
                pcar[t] = p[n:, cols].astype(pcar.dtype)
        v = as_bf16(v32)
        if last:
            n = done_rows
            rcar[...] = jnp.broadcast_to(inv[n:], rcar.shape)
            vcar[...] = v32
        pb = jnp.concatenate([load(pbuf.at[u, t, pl.ds(0, n)]) for t in range(tiles)], axis=1)
        o = jnp.dot(pb, v, preferred_element_type=jnp.float32)
        ob[i, r, pl.ds(0, n)] = (o * inv[:n]).astype(ob.dtype)
        if last:
            for t in range(tiles):
                ocar[t] = jnp.dot(load(pbuf.at[u, t, pl.ds(n, _RAW_ROWS)]), v[t * _LANES:(t + 1) * _LANES],
                                  preferred_element_type=jnp.float32)

    def finish_head(j, pieces=1, after_piece=lambda *_: None):
        r, i = where_is(j)
        pb = jnp.concatenate([load(pcar.at[t]) for t in range(tiles)], axis=1)
        o = jnp.dot(pb, as_bf16(vcar[...]), preferred_element_type=jnp.float32)
        raw = functools.reduce(jnp.add, [ocar[t] + ocar[t + 1] for t in range(0, tiles, 2)])
        ob[i, r, pl.ds(done_rows, _RAW_ROWS)] = (raw * rcar[pl.ds(0, _RAW_ROWS)]).astype(ob.dtype)
        after_piece(j, done_rows, _RAW_ROWS)
        o = (o * rcar[pl.ds(_RAW_ROWS, _CARRY_ROWS)]).astype(ob.dtype)
        n = _CARRY_ROWS // pieces
        for row0 in range(0, _CARRY_ROWS, n):
            ob[i, r, pl.ds(keep + row0, n)] = o[row0:row0 + n]
            after_piece(j, keep + row0, n)

    def run_segment(si, lo):
        size, count, per_group = segs[si]
        h0 = starts[si]
        hi = lo + count * per_group
        final = si == len(segs) - 1
        assert final or h0 + size * count <= _WRITE_FROM
        for it in range(count):
            issued = lo + it * per_group
            assert min(n_heads, issued + per_group) - _RING <= h0 + it * size
            assert min(issued, max(issued - _V_LAG, first_split)) >= h0 + (it + 1) * size
            assert (h0 + it * size) % _RING + size <= _RING

        def group(it, slot0):
            base = h0 + it * size
            dst = ib.at[pl.ds(slot0, size)]
            pltpu.make_async_copy(dst, dst, sem.at[gbase[si] + it]).wait()
            if h0 > 0:
                finish_head(base - 1)
            for g in range(size):
                j, slot = base + g, slot0 + g
                reads = []
                for t in range((per_group * g) // size, (per_group * (g + 1)) // size):
                    idx = lo + it * per_group + t
                    if si < _SPLIT_FROM:
                        reads.append(functools.partial(start_reads, (1, 0, 2), idx, lo, hi))
                    else:
                        reads += [functools.partial(start_part, idx, lo, hi, part) for part in range(_READ_SPLIT)]
                early = 2 * len(reads) // 3
                k = load(ib.at[slot, 1])
                for start in reads[:early]:
                    start()
                if size >= regions and (size - 1 - g) % _WRITE_EVERY == 0:
                    back = min(_WRITE_EVERY, g + 1)
                    w0, w1 = bulk_before(j - back), bulk_before(j)
                    for t in range(max(_WRITES_PER_HEAD * back, chunks) if final else 1):
                        pl.when(w0 + t < w1)(functools.partial(start_bulk_write, w0 + t))
                    for done in range(n_heads - size + g - back, n_heads - size + g):
                        if final and done >= n_heads - regions:
                            pl.when(it == count - 1)(functools.partial(start_head_write, done))
                v32 = load_words(ib.at[slot, 2])
                q_top = load(ib.at[slot, 0, pl.ds(0, seq // 2)])
                for start in reads[early:]:
                    start()
                q_bottom = load(ib.at[slot, 0, pl.ds(seq // 2, seq // 2)])
                head(jnp.concatenate([q_top, q_bottom], axis=0), k, v32, g % 2, j, g == size - 1)
            return slot_of(base + size, h0 + size, h0 + size * (count + 1))

        if count == 1:
            group(0, h0 % _RING)
        else:
            lax.fori_loop(0, count, group, h0 % _RING)
        return hi

    @pl.when(pl.program_id(0) == 0)
    def _():
        for j in range(_FIRST_READS):
            start_reads((1, 0, 2), j, None, None)

    @pl.when(pl.program_id(0) == 1)
    def _():
        issued = _FIRST_READS
        for si in range(len(segs)):
            issued = run_segment(si, issued)
        assert issued - _V_LAG >= n_heads and bulk_before(n_heads - 1) == n_bulk
        start_head_write(n_heads - 1, 0, done_rows)
        finish_head(n_heads - 1, _LAST_PIECES, start_head_write)
        pltpu.make_async_copy(o_hbm, o_hbm, write_sem).wait()


@jax.jit
def pallas_standalone__mha_softmax__near_ridge_kernel(
    q: jax.Array,
    k: jax.Array,
    v: jax.Array,
):
    B, H, S, D = q.shape
    per_region = B * H // _REGIONS
    shape = (_REGIONS, per_region, S, D)
    n_groups = sum(count for _, count, _ in _SEGMENTS)
    out = pl.pallas_call(
        functools.partial(_attn_kernel, scale=D ** -0.5),
        grid=(2,),
        in_specs=[pl.BlockSpec(memory_space=pl.ANY)] * 3,
        out_specs=pl.BlockSpec(memory_space=pl.ANY),
        out_shape=jax.ShapeDtypeStruct(shape, q.dtype),
        scratch_shapes=[
            pltpu.VMEM((_RING, 3, S, D), q.dtype),
            pltpu.VMEM((per_region, _REGIONS, S, D), q.dtype),
            pltpu.VMEM((2, S // _LANES, S, _LANES), q.dtype),
            pltpu.VMEM((S // _LANES, _CARRY_ROWS, _LANES), q.dtype),
            pltpu.VMEM((_RAW_ROWS + _CARRY_ROWS, D), jnp.float32),
            pltpu.VMEM((S // 2, D), jnp.uint32),
            pltpu.VMEM((S // _LANES, _RAW_ROWS, D), jnp.float32),
            pltpu.SemaphoreType.DMA((n_groups + 1,)),
        ],
        compiler_params=pltpu.CompilerParams(
            dimension_semantics=("arbitrary",),
            vmem_limit_bytes=110 * 1024 * 1024,
            disable_bounds_checks=True,
            disable_semaphore_checks=True,
        ),
    )(q.reshape(shape), k.reshape(shape), v.reshape(shape))
    return out.reshape(B, H, S, D)
```

```python
import functools

import jax
import jax.numpy as jnp
from jax import lax
import jax.experimental.pallas as pl
import jax.experimental.pallas.tpu as pltpu

_LOG2E = 1.4426950408889634
_NT = (((1,), (1,)), ((), ()))
_LANES = 128

_SEGMENTS = ((1, 1, 2), (1, 2, 2), (2, 2, 3), (3, 1, 4), (4, 2, 6), (8, 2, 12), (14, 3, 19), (30, 6, 41))
_RING = 136
_FIRST_READS = 3
_SPLIT_FROM = 3
_READ_SPLIT = 4
_V_LAG = 3
_REGIONS = 4
_WRITE_ROWS = 128
_WRITE_FROM = 184
_WRITES_PER_HEAD = 4
_WRITE_EVERY = 2
_CARRY_ROWS = 128
_RAW_ROWS = 32
_Q_TOP_ROWS = 288
_LAST_PIECES = 4


def _shift(x, pow2):
    if isinstance(x, int):
        return x // pow2
    return lax.shift_right_arithmetic(x, pow2.bit_length() - 1)


def _attn_kernel(q_hbm, k_hbm, v_hbm, o_hbm, ib, ob, pbuf, pcar, rcar, vcar, ocar, sem, *, scale):
    regions, per_region, seq, _ = q_hbm.shape
    n_heads = regions * per_region
    tiles = seq // _LANES
    keep = seq - _CARRY_ROWS
    done_rows = keep - _RAW_ROWS
    c = scale * _LOG2E
    hbms = (q_hbm, k_hbm, v_hbm)
    segs = _SEGMENTS

    starts, gbase = [], []
    h = n_groups = 0
    for size, count, _ in segs:
        starts.append(h)
        gbase.append(n_groups)
        h += size * count
        n_groups += count
    assert h == n_heads <= 2 * _RING and segs[0][1] == 1
    write_sem = sem.at[n_groups]
    first_split = _FIRST_READS + sum(count * per_group for _, count, per_group in segs[:_SPLIT_FROM])

    def where_is(j):
        return j & (regions - 1), _shift(j, regions)

    def group_of(j, lo, hi):
        res = None
        for s0, g0, (size, count, _) in zip(starts, gbase, segs):
            if s0 + size * count <= lo or s0 >= hi:
                continue
            magic = -(-(1 << 16) // size)
            assert all((x * magic) >> 16 == x // size for x in range(n_heads))
            g = g0 + _shift((j - s0) * magic, 1 << 16)
            res = g if res is None else jnp.where(j >= s0, g, res)
        return res

    def slot_of(j, lo, hi):
        if hi <= _RING:
            return j
        if lo >= _RING:
            return j - _RING
        return jnp.where(j >= _RING, j - _RING, j)

    def start_reads(arrays, j, lo, hi, part=0, split=1, priority=0):
        first = first_split if split > 1 else 0
        if isinstance(j, int):
            lo, hi = j, j + 1

        def start():
            group, slot = group_of(j, max(lo, first), min(hi, n_heads)), slot_of(j, lo, hi)
            r, i = where_is(j)
            rows = pl.ds(part * (seq // split), seq // split)
            for a in arrays:
                pltpu.make_async_copy(hbms[a].at[r, i, rows], ib.at[slot, a, rows], sem.at[group]).start(
                    priority=priority)

        if first <= lo and hi <= n_heads:
            start()
        elif not isinstance(j, int):
            pl.when(jnp.logical_and(j >= first, j < n_heads))(start)

    def start_part(j, lo, hi, part):
        start_reads((1, 0), j, lo, hi, part, _READ_SPLIT, 1)
        start_reads((2,), j - _V_LAG, lo - _V_LAG, hi - _V_LAG, part, _READ_SPLIT, 0)

    chunks = seq // _WRITE_ROWS
    n_bulk = (per_region - 1) * chunks

    def start_bulk_write(u):
        i = _shift(u, chunks)
        row0 = (u & (chunks - 1)) * _WRITE_ROWS
        if not isinstance(row0, int):
            row0 = pl.multiple_of(row0, _WRITE_ROWS)
        rows = pl.ds(row0, _WRITE_ROWS)
        pltpu.make_async_copy(ob.at[i, :, rows], o_hbm.at[:, i, rows], write_sem).start()

    def start_head_write(j, row0=0, n=seq):
        r, i = where_is(j)
        rows = pl.ds(row0, n)
        pltpu.make_async_copy(ob.at[i, r, rows], o_hbm.at[r, i, rows], write_sem).start()

    def bulk_before(j):
        mx, mn = (max, min) if isinstance(j, int) else (jnp.maximum, jnp.minimum)
        return mx(mn(mn(_WRITES_PER_HEAD * (j - _WRITE_FROM), _shift(j, regions) * chunks), n_bulk), 0)

    def load_words(view):
        return view.bitcast(jnp.uint32)[...]

    def as_bf16(x):
        return pltpu.bitcast(x, jnp.bfloat16)

    def load(view):
        return as_bf16(load_words(view))

    def head(q, k, v32, u, j, last):
        n = keep if last else seq
        r, i = where_is(j)
        s = lax.dot_general(q, k, _NT, preferred_element_type=jnp.float32)
        m = jnp.max(s, axis=-1, keepdims=True)
        p = jnp.exp2((s - m) * c)
        l = jnp.sum(p, axis=-1, keepdims=True)
        inv = pl.reciprocal(l, approx=True)
        inv = inv * (2.0 - l * inv)
        for t in range(tiles):
            cols = slice(t * _LANES, (t + 1) * _LANES)
            pbuf[u, t, pl.ds(0, n)] = p[:n, cols].astype(pbuf.dtype)
            if last:
                pcar[t] = p[n:, cols].astype(pcar.dtype)
        v = as_bf16(v32)
        if last:
            n = done_rows
            rcar[...] = jnp.broadcast_to(inv[n:], rcar.shape)
            vcar[...] = v32
        pb = jnp.concatenate([load(pbuf.at[u, t, pl.ds(0, n)]) for t in range(tiles)], axis=1)
        o = jnp.dot(pb, v, preferred_element_type=jnp.float32)
        ob[i, r, pl.ds(0, n)] = (o * inv[:n]).astype(ob.dtype)
        if last:
            for t in range(tiles):
                ocar[t] = jnp.dot(load(pbuf.at[u, t, pl.ds(n, _RAW_ROWS)]), v[t * _LANES:(t + 1) * _LANES],
                                  preferred_element_type=jnp.float32)

    def finish_head(j, pieces=1, after_piece=lambda *_: None):
        r, i = where_is(j)
        pb = jnp.concatenate([load(pcar.at[t]) for t in range(tiles)], axis=1)
        o = jnp.dot(pb, as_bf16(vcar[...]), preferred_element_type=jnp.float32)
        raw = functools.reduce(jnp.add, [ocar[t] + ocar[t + 1] for t in range(0, tiles, 2)])
        ob[i, r, pl.ds(done_rows, _RAW_ROWS)] = (raw * rcar[pl.ds(0, _RAW_ROWS)]).astype(ob.dtype)
        after_piece(j, done_rows, _RAW_ROWS)
        o = (o * rcar[pl.ds(_RAW_ROWS, _CARRY_ROWS)]).astype(ob.dtype)
        n = _CARRY_ROWS // pieces
        for row0 in range(0, _CARRY_ROWS, n):
            ob[i, r, pl.ds(keep + row0, n)] = o[row0:row0 + n]
            after_piece(j, keep + row0, n)

    def run_segment(si, lo):
        size, count, per_group = segs[si]
        h0 = starts[si]
        hi = lo + count * per_group
        final = si == len(segs) - 1
        assert final or h0 + size * count <= _WRITE_FROM
        for it in range(count):
            issued = lo + it * per_group
            assert min(n_heads, issued + per_group) - _RING <= h0 + it * size
            assert min(issued, max(issued - _V_LAG, first_split)) >= h0 + (it + 1) * size
            assert (h0 + it * size) % _RING + size <= _RING

        def group(it, slot0):
            base = h0 + it * size
            dst = ib.at[pl.ds(slot0, size)]
            pltpu.make_async_copy(dst, dst, sem.at[gbase[si] + it]).wait()
            if h0 > 0:
                finish_head(base - 1)
            for g in range(size):
                j, slot = base + g, slot0 + g
                reads = []
                for t in range((per_group * g) // size, (per_group * (g + 1)) // size):
                    idx = lo + it * per_group + t
                    if si < _SPLIT_FROM:
                        reads.append(functools.partial(start_reads, (1, 0, 2), idx, lo, hi))
                    else:
                        reads += [functools.partial(start_part, idx, lo, hi, part) for part in range(_READ_SPLIT)]
                early = 2 * len(reads) // 3
                k = load(ib.at[slot, 1])
                for start in reads[:early]:
                    start()
                if size >= regions and (size - 1 - g) % _WRITE_EVERY == 0:
                    back = min(_WRITE_EVERY, g + 1)
                    w0, w1 = bulk_before(j - back), bulk_before(j)
                    for t in range(max(_WRITES_PER_HEAD * back, chunks)):
                        pl.when(w0 + t < w1)(functools.partial(start_bulk_write, w0 + t))
                    for done in range(n_heads - size + g - back, n_heads - size + g):
                        if final and done >= n_heads - regions:
                            pl.when(it == count - 1)(functools.partial(start_head_write, done))
                v32 = load_words(ib.at[slot, 2])
                q_top = load(ib.at[slot, 0, pl.ds(0, _Q_TOP_ROWS)])
                for start in reads[early:]:
                    start()
                q_bottom = load(ib.at[slot, 0, pl.ds(_Q_TOP_ROWS, seq - _Q_TOP_ROWS)])
                head(jnp.concatenate([q_top, q_bottom], axis=0), k, v32, g % 2, j, g == size - 1)
            return slot_of(base + size, h0 + size, h0 + size * (count + 1))

        if count == 1:
            group(0, h0 % _RING)
        else:
            lax.fori_loop(0, count, group, h0 % _RING)
        return hi

    @pl.when(pl.program_id(0) == 0)
    def _():
        for j in range(_FIRST_READS):
            start_reads((1, 0, 2), j, None, None)

    @pl.when(pl.program_id(0) == 1)
    def _():
        issued = _FIRST_READS
        for si in range(len(segs)):
            issued = run_segment(si, issued)
        assert issued - _V_LAG >= n_heads and bulk_before(n_heads - 1) == n_bulk
        start_head_write(n_heads - 1, 0, done_rows)
        finish_head(n_heads - 1, _LAST_PIECES, start_head_write)
        pltpu.make_async_copy(o_hbm, o_hbm, write_sem).wait()


@jax.jit
def pallas_standalone__mha_softmax__near_ridge_kernel(
    q: jax.Array,
    k: jax.Array,
    v: jax.Array,
):
    B, H, S, D = q.shape
    per_region = B * H // _REGIONS
    shape = (_REGIONS, per_region, S, D)
    n_groups = sum(count for _, count, _ in _SEGMENTS)
    out = pl.pallas_call(
        functools.partial(_attn_kernel, scale=D ** -0.5),
        grid=(2,),
        in_specs=[pl.BlockSpec(memory_space=pl.ANY)] * 3,
        out_specs=pl.BlockSpec(memory_space=pl.ANY),
        out_shape=jax.ShapeDtypeStruct(shape, q.dtype),
        scratch_shapes=[
            pltpu.VMEM((_RING, 3, S, D), q.dtype),
            pltpu.VMEM((per_region, _REGIONS, S, D), q.dtype),
            pltpu.VMEM((2, S // _LANES, S, _LANES), q.dtype),
            pltpu.VMEM((S // _LANES, _CARRY_ROWS, _LANES), q.dtype),
            pltpu.VMEM((_RAW_ROWS + _CARRY_ROWS, D), jnp.float32),
            pltpu.VMEM((S // 2, D), jnp.uint32),
            pltpu.VMEM((S // _LANES, _RAW_ROWS, D), jnp.float32),
            pltpu.SemaphoreType.DMA((n_groups + 1,)),
        ],
        compiler_params=pltpu.CompilerParams(
            dimension_semantics=("arbitrary",),
            vmem_limit_bytes=110 * 1024 * 1024,
            disable_bounds_checks=True,
            disable_semaphore_checks=True,
        ),
    )(q.reshape(shape), k.reshape(shape), v.reshape(shape))
    return out.reshape(B, H, S, D)
```
